```python
import os as _os
_os.environ.setdefault("JAX_PLATFORMS", "cpu")
import jax
import jax.numpy as jnp

def _softmax(x, axis=-1):
    return jax.nn.softmax(x, axis=axis)
def _gelu(x):
    return jax.nn.gelu(x, approximate=True)
def _silu(x):
    return jax.nn.silu(x)
def _sigmoid(x):
    return jax.nn.sigmoid(x)
def _layernorm(x, axis=-1, eps=1e-5):
    m = jnp.mean(x, axis=axis, keepdims=True)
    v = jnp.var(x, axis=axis, keepdims=True)
    return (x - m) / jnp.sqrt(v + eps)
def _scatter_add(tgt, idx, src, axis=0):
    return tgt.at[idx].add(src)
def _segment_sum(src, seg, n):
    return jax.ops.segment_sum(src, seg, n)
class _Rng:
    def __init__(self, key):
        self._k = key
    def _next(self):
        self._k, sub = jax.random.split(self._k)
        return sub
    def normal(self, shape):
        return jax.random.normal(self._next(), shape, dtype=jnp.bfloat16)
    def randint(self, lo, hi, shape):
        return jax.random.randint(self._next(), shape, lo, hi, dtype=jnp.int32)
    def uniform(self, shape, lo=0.0, hi=1.0):
        return jax.random.uniform(self._next(), shape, jnp.bfloat16, lo, hi)
    def permutation(self, n):
        return jax.random.permutation(self._next(), n)


kernel_name = 'standalone__dense_activation_gelu__prompt'

def setup_inputs():
    _rng = _Rng(jax.random.key(int.from_bytes(__import__("os").urandom(4), "little")))
    _w = (lambda a: (lambda t: t.astype(jnp.bfloat16) if jnp.issubdtype(t.dtype, jnp.floating) else t)(jnp.asarray(a)))
    B, S, D, F = 1, 2048, 640, 1728
    return {
        "x": _w((lambda *s: _rng.normal(s) * 0.05)(B, S, D)),
        "w1": _w((lambda *s: _rng.normal(s) * 0.05)(D, F) * (D ** -0.5)),
        "b1": _w((lambda *s: _rng.normal(s) * 0.05)(F) * 0.01),
        "w2": _w((lambda *s: _rng.normal(s) * 0.05)(F, D) * (F ** -0.5)),
        "b2": _w((lambda *s: _rng.normal(s) * 0.05)(D) * 0.01),
    }

def reference(x, w1, b1, w2, b2):
    h = jnp.einsum("bsd,df->bsf", x, w1) + b1
    h = _gelu(h)
    return jnp.einsum("bsf,fd->bsd", h, w2) + b2
```

```python
import functools
import numpy as np
import jax
import jax.numpy as jnp
import jax.experimental.pallas as pl
import jax.experimental.pallas.tpu as pltpu


def _gelu_tanh(h):
    c0 = np.float32(np.sqrt(2.0 / np.pi))
    c1 = np.float32(0.044715 * np.sqrt(2.0 / np.pi))
    inner = h * (c0 + c1 * (h * h))
    hh = 0.5 * h
    return hh + hh * jnp.tanh(inner)


def _ffn_kernel(x_ref, w1_ref, b1_ref, w2_ref, b2_ref, o_ref):
    x = x_ref[...]
    h = jnp.dot(x, w1_ref[...], preferred_element_type=jnp.float32)
    h = h + b1_ref[...].astype(jnp.float32)
    g = _gelu_tanh(h).astype(jnp.bfloat16)
    o = jnp.dot(g, w2_ref[...], preferred_element_type=jnp.float32)
    o = o + b2_ref[...].astype(jnp.float32)
    o_ref[...] = o.astype(o_ref.dtype)


@jax.jit
def pallas_standalone__dense_activation_gelu__prompt_kernel(
    x: jax.Array,
    w1: jax.Array,
    b1: jax.Array,
    w2: jax.Array,
    b2: jax.Array,
):
    B, S, D = x.shape
    F = w1.shape[1]
    M = B * S
    TM = 512
    x2 = x.reshape(M, D)
    b1r = b1.reshape(1, F)
    b2r = b2.reshape(1, D)

    out = pl.pallas_call(
        _ffn_kernel,
        grid=(M // TM,),
        in_specs=[
            pl.BlockSpec((TM, D), lambda i: (i, 0)),
            pl.BlockSpec((D, F), lambda i: (0, 0)),
            pl.BlockSpec((1, F), lambda i: (0, 0)),
            pl.BlockSpec((F, D), lambda i: (0, 0)),
            pl.BlockSpec((1, D), lambda i: (0, 0)),
        ],
        out_specs=pl.BlockSpec((TM, D), lambda i: (i, 0)),
        out_shape=jax.ShapeDtypeStruct((M, D), x.dtype),
        compiler_params=pltpu.CompilerParams(
            dimension_semantics=("arbitrary",),
            vmem_limit_bytes=64 * 1024 * 1024,
        ),
    )(x2, w1, b1r, w2, b2r)
    return out.reshape(B, S, D)
```

```python
import numpy as np
import jax
import jax.numpy as jnp
import jax.experimental.pallas as pl
import jax.experimental.pallas.tpu as pltpu

ROW_TILES = [512, 512, 512, 256, 128, 128]
W1_CUTS = [0, 256, 768, 1728]
VMEM_MB = 100


def _gelu_tanh(h):
    c0 = np.float32(np.sqrt(2.0 / np.pi))
    c1 = np.float32(0.044715 * np.sqrt(2.0 / np.pi))
    inner = h * (c0 + c1 * (h * h))
    hh = 0.5 * h
    return hh + hh * jnp.tanh(inner)


def _dot_nt(a, bt):
    return jax.lax.dot_general(a, bt, (((1,), (1,)), ((), ())),
                               preferred_element_type=jnp.float32)


def _make_kernel(M, D, F, row_tiles, w1_cuts):
    row_starts = [int(v) for v in np.cumsum([0] + list(row_tiles))]
    assert row_starts[-1] == M
    n_tiles = len(row_tiles)
    n_w1 = len(w1_cuts) - 1
    tm0 = row_tiles[0]

    def kernel(x_hbm, w1t_hbm, b1_hbm, w2_hbm, b2_hbm, o_hbm,
               xv, w1v, w2v, b1v, b2v, ov, gv,
               sem_x, sem_w1, sem_w2, sem_b, sem_o):

        def x_copy(r0, r1, s):
            return pltpu.make_async_copy(
                x_hbm.at[pl.ds(r0, r1 - r0)], xv.at[pl.ds(r0, r1 - r0)], sem_x.at[s])

        def w1_copy(c):
            c0, c1 = w1_cuts[c], w1_cuts[c + 1]
            return pltpu.make_async_copy(
                w1t_hbm.at[pl.ds(c0, c1 - c0)], w1v.at[pl.ds(c0, c1 - c0)], sem_w1.at[c])

        def w2_copy():
            return pltpu.make_async_copy(w2_hbm, w2v, sem_w2.at[0])

        def b1_copy():
            return pltpu.make_async_copy(b1_hbm, b1v, sem_b.at[0])

        def b2_copy():
            return pltpu.make_async_copy(b2_hbm, b2v, sem_b.at[1])

        def o_copy(t):
            r0, r1 = row_starts[t], row_starts[t + 1]
            return pltpu.make_async_copy(
                ov.at[pl.ds(r0, r1 - r0)], o_hbm.at[pl.ds(r0, r1 - r0)], sem_o.at[t])

        x_copy(0, tm0, 0).start()
        w1_copy(0).start()
        b1_copy().start()
        for c in range(1, n_w1):
            w1_copy(c).start()
        w2_copy().start()
        b2_copy().start()
        x_copy(tm0, M, 1).start()

        x_copy(0, tm0, 0).wait()
        b1_copy().wait()
        for c in range(n_w1):
            c0, c1 = w1_cuts[c], w1_cuts[c + 1]
            w1_copy(c).wait()
            h = _dot_nt(xv[0:tm0, :], w1v[c0:c1, :])
            h = h + b1v[c0:c1].astype(jnp.float32)[None, :]
            gv[:, c0:c1] = _gelu_tanh(h).astype(gv.dtype)
        w2_copy().wait()
        b2_copy().wait()
        o = jnp.dot(gv[...], w2v[...], preferred_element_type=jnp.float32)
        o = o + b2v[...].astype(jnp.float32)[None, :]
        ov[0:tm0, :] = o.astype(ov.dtype)
        o_copy(0).start()

        x_copy(tm0, M, 1).wait()
        for t in range(1, n_tiles):
            r0, r1 = row_starts[t], row_starts[t + 1]
            h = _dot_nt(xv[r0:r1, :], w1v[...])
            h = h + b1v[...].astype(jnp.float32)[None, :]
            g = _gelu_tanh(h).astype(jnp.bfloat16)
            o = jnp.dot(g, w2v[...], preferred_element_type=jnp.float32)
            o = o + b2v[...].astype(jnp.float32)[None, :]
            ov[r0:r1, :] = o.astype(ov.dtype)
            o_copy(t).start()

        for t in range(n_tiles):
            o_copy(t).wait()

    return kernel, n_tiles, n_w1, tm0


@jax.jit
def pallas_standalone__dense_activation_gelu__prompt_kernel(x, w1, b1, w2, b2):
    B, S, D = x.shape
    F = w1.shape[1]
    M = B * S
    x2 = x.reshape(M, D)
    w1t = w1.T
    kernel, n_tiles, n_w1, tm0 = _make_kernel(M, D, F, ROW_TILES, W1_CUTS)
    anyspec = pl.BlockSpec(memory_space=pl.ANY)

    out = pl.pallas_call(
        kernel,
        in_specs=[anyspec, anyspec, anyspec, anyspec, anyspec],
        out_specs=anyspec,
        out_shape=jax.ShapeDtypeStruct((M, D), x.dtype),
        scratch_shapes=[
            pltpu.VMEM((M, D), x.dtype),
            pltpu.VMEM((F, D), w1.dtype),
            pltpu.VMEM((F, D), w2.dtype),
            pltpu.VMEM((F,), b1.dtype),
            pltpu.VMEM((D,), b2.dtype),
            pltpu.VMEM((M, D), x.dtype),
            pltpu.VMEM((tm0, F), jnp.bfloat16),
            pltpu.SemaphoreType.DMA((2,)),
            pltpu.SemaphoreType.DMA((n_w1,)),
            pltpu.SemaphoreType.DMA((1,)),
            pltpu.SemaphoreType.DMA((2,)),
            pltpu.SemaphoreType.DMA((n_tiles,)),
        ],
        compiler_params=pltpu.CompilerParams(
            vmem_limit_bytes=int(VMEM_MB * 1024 * 1024),
        ),
    )(x2, w1t, b1, w2, b2)
    return out.reshape(B, S, D)
```

```python
import numpy as np
import jax
import jax.numpy as jnp
import jax.experimental.pallas as pl
import jax.experimental.pallas.tpu as pltpu

_ROW_TILES = (512, 512, 512, 256, 128, 128)
_W1_CUTS = (0, 256, 768, 1728)
_VMEM_LIMIT_BYTES = 100 * 1024 * 1024


def _gelu_tanh(h):
    c0 = np.float32(np.sqrt(2.0 / np.pi))
    c1 = np.float32(0.044715 * np.sqrt(2.0 / np.pi))
    inner = h * (c0 + c1 * (h * h))
    hh = 0.5 * h
    return hh + hh * jnp.tanh(inner)


def _dot_nt(a, bt):
    return jax.lax.dot_general(a, bt, (((1,), (1,)), ((), ())),
                               preferred_element_type=jnp.float32)


def _make_kernel(M, F, row_tiles, w1_cuts):
    row_starts = [int(v) for v in np.cumsum([0] + list(row_tiles))]
    assert row_starts[-1] == M and w1_cuts[0] == 0 and w1_cuts[-1] == F
    n_tiles = len(row_tiles)
    n_w1 = len(w1_cuts) - 1
    tm0 = row_tiles[0]
    hm = tm0 // 2
    x_pieces = ((0, tm0), (tm0, M))

    def kernel(x_hbm, w1t_hbm, b1_hbm, w2_hbm, b2_hbm, o_hbm,
               xv, w1v, w2v, b1v, b2v, ov, gv,
               sem_x, sem_w1, sem_w2, sem_b, sem_o):

        def x_copy(p):
            r0, r1 = x_pieces[p]
            return pltpu.make_async_copy(
                x_hbm.at[pl.ds(r0, r1 - r0)], xv.at[pl.ds(r0, r1 - r0)],
                sem_x.at[p])

        def w1_copy(c):
            c0, c1 = w1_cuts[c], w1_cuts[c + 1]
            return pltpu.make_async_copy(
                w1t_hbm.at[pl.ds(c0, c1 - c0)], w1v.at[pl.ds(c0, c1 - c0)],
                sem_w1.at[c])

        def w2_copy():
            return pltpu.make_async_copy(w2_hbm, w2v, sem_w2.at[0])

        def b1_copy():
            return pltpu.make_async_copy(b1_hbm, b1v, sem_b.at[0])

        def b2_copy():
            return pltpu.make_async_copy(b2_hbm, b2v, sem_b.at[1])

        def o_copy(t):
            r0, r1 = row_starts[t], row_starts[t + 1]
            return pltpu.make_async_copy(
                ov.at[pl.ds(r0, r1 - r0)], o_hbm.at[pl.ds(r0, r1 - r0)],
                sem_o.at[t])

        def ffn1(r0, r1, c0, c1):
            h = _dot_nt(xv[r0:r1, :], w1v[c0:c1, :])
            h = h + b1v[c0:c1].astype(jnp.float32)[None, :]
            return _gelu_tanh(h).astype(jnp.bfloat16)

        def ffn2(g):
            o = jnp.dot(g, w2v[...], preferred_element_type=jnp.float32)
            o = o + b2v[...].astype(jnp.float32)[None, :]
            return o.astype(ov.dtype)

        x_copy(0).start()
        w1_copy(0).start()
        b1_copy().start()
        for c in range(1, n_w1):
            w1_copy(c).start()
        w2_copy().start()
        b2_copy().start()
        x_copy(1).start()

        x_copy(0).wait()
        b1_copy().wait()
        w1_copy(0).wait()
        c0, c1 = w1_cuts[0], w1_cuts[1]
        gv[0:hm, c0:c1] = ffn1(0, hm, c0, c1)
        gv[hm:tm0, c0:c1] = ffn1(hm, tm0, c0, c1)
        for c in range(1, n_w1):
            c0, c1 = w1_cuts[c], w1_cuts[c + 1]
            w1_copy(c).wait()
            gv[:, c0:c1] = ffn1(0, tm0, c0, c1)
        w2_copy().wait()
        b2_copy().wait()
        ov[0:hm, :] = ffn2(gv[0:hm, :])
        ov[hm:tm0, :] = ffn2(gv[hm:tm0, :])
        o_copy(0).start()

        x_copy(1).wait()
        for t in range(1, n_tiles):
            r0, r1 = row_starts[t], row_starts[t + 1]
            ov[r0:r1, :] = ffn2(ffn1(r0, r1, 0, F))
            o_copy(t).start()

        for t in range(n_tiles):
            o_copy(t).wait()

    return kernel, n_tiles, n_w1, tm0


@jax.jit
def pallas_standalone__dense_activation_gelu__prompt_kernel(
    x: jax.Array,
    w1: jax.Array,
    b1: jax.Array,
    w2: jax.Array,
    b2: jax.Array,
):
    B, S, D = x.shape
    F = w1.shape[1]
    M = B * S
    kernel, n_tiles, n_w1, tm0 = _make_kernel(M, F, _ROW_TILES, _W1_CUTS)
    anyspec = pl.BlockSpec(memory_space=pl.ANY)

    out = pl.pallas_call(
        kernel,
        in_specs=[anyspec, anyspec, anyspec, anyspec, anyspec],
        out_specs=anyspec,
        out_shape=jax.ShapeDtypeStruct((M, D), x.dtype),
        scratch_shapes=[
            pltpu.VMEM((M, D), x.dtype),
            pltpu.VMEM((F, D), w1.dtype),
            pltpu.VMEM((F, D), w2.dtype),
            pltpu.VMEM((F,), b1.dtype),
            pltpu.VMEM((D,), b2.dtype),
            pltpu.VMEM((M, D), x.dtype),
            pltpu.VMEM((tm0, F), jnp.bfloat16),
            pltpu.SemaphoreType.DMA((2,)),
            pltpu.SemaphoreType.DMA((n_w1,)),
            pltpu.SemaphoreType.DMA((1,)),
            pltpu.SemaphoreType.DMA((2,)),
            pltpu.SemaphoreType.DMA((n_tiles,)),
        ],
        compiler_params=pltpu.CompilerParams(
            vmem_limit_bytes=_VMEM_LIMIT_BYTES,
        ),
    )(x.reshape(M, D), w1.T, b1, w2, b2)
    return out.reshape(B, S, D)
```
